```python
import os as _os
_os.environ.setdefault("JAX_PLATFORMS", "cpu")
import jax
import jax.numpy as jnp

def _softmax(x, axis=-1):
    return jax.nn.softmax(x, axis=axis)
def _gelu(x):
    return jax.nn.gelu(x, approximate=True)
def _silu(x):
    return jax.nn.silu(x)
def _sigmoid(x):
    return jax.nn.sigmoid(x)
def _layernorm(x, axis=-1, eps=1e-5):
    m = jnp.mean(x, axis=axis, keepdims=True)
    v = jnp.var(x, axis=axis, keepdims=True)
    return (x - m) / jnp.sqrt(v + eps)
def _scatter_add(tgt, idx, src, axis=0):
    return tgt.at[idx].add(src)
def _segment_sum(src, seg, n):
    return jax.ops.segment_sum(src, seg, n)
class _Rng:
    def __init__(self, key):
        self._k = key
    def _next(self):
        self._k, sub = jax.random.split(self._k)
        return sub
    def normal(self, shape):
        return jax.random.normal(self._next(), shape, dtype=jnp.bfloat16)
    def randint(self, lo, hi, shape):
        return jax.random.randint(self._next(), shape, lo, hi, dtype=jnp.int32)
    def uniform(self, shape, lo=0.0, hi=1.0):
        return jax.random.uniform(self._next(), shape, jnp.bfloat16, lo, hi)
    def permutation(self, n):
        return jax.random.permutation(self._next(), n)


kernel_name = 'gated_mix__linear_attn_block__swiglu_ffn__prompt'

def setup_inputs():
    _rng = _Rng(jax.random.key(int.from_bytes(__import__("os").urandom(4), "little")))
    _w = (lambda a: (lambda t: t.astype(jnp.bfloat16) if jnp.issubdtype(t.dtype, jnp.floating) else t)(jnp.asarray(a)))
    def _A_setup():
        B, S, D = 1, 2048, 512
        return {
            "x": _w((lambda *s: _rng.normal(s) * 0.05)(B, S, D)),
            "wqkv": _w((lambda *s: _rng.normal(s) * 0.8)(D, 3 * D)),
            "wo": _w((lambda *s: _rng.normal(s) * 0.05)(D, D)),
        }
    _A_in = _A_setup()

    def _B_setup():
        B, S, D, F = 1, 2048, 512, 1792
        return {
            "x": _w((lambda *s: _rng.normal(s) * 0.05)(B, S, D)),
            "w_gate": _w((lambda *s: _rng.normal(s) * 0.1)(D, F)),
            "w_up": _w((lambda *s: _rng.normal(s) * 0.1)(D, F)),
            "w_down": _w((lambda *s: _rng.normal(s) * 0.1)(F, D)),
        }
    _B_in = _B_setup()

    return {
        "A_x": _A_in["x"],
        "A_wqkv": _A_in["wqkv"],
        "A_wo": _A_in["wo"],
        "B_x": _B_in["x"],
        "B_w_gate": _B_in["w_gate"],
        "B_w_up": _B_in["w_up"],
        "B_w_down": _B_in["w_down"],
        "gate_w": _w((lambda *s: _rng.normal(s) * 0.05)(512) * 16.0),
    }

def reference(A_x, A_wqkv, A_wo, B_x, B_w_gate, B_w_up, B_w_down, gate_w):
    def _A_ref(x, wqkv, wo):
        B, S, D = x.shape
        H = 32; Dh = D // H
        qkv = (lambda x, *d: x.transpose(*d))((x @ wqkv).reshape(B, S, 3, H, Dh), 2, 0, 3, 1, 4)
        q, k, v = qkv[0], qkv[1], qkv[2]
        phi = lambda t: jnp.where(t > 0, t + 1, jnp.exp(t)) + 1e-6
        pq, pk = phi(q), phi(k)
        kv = jnp.einsum("bhsd,bhse->bhde", pk, v)
        z = jnp.einsum("bhsd->bhd", pk)
        num = jnp.einsum("bhqd,bhde->bhqe", pq, kv)
        den = jnp.einsum("bhqd,bhd->bhq", pq, z)[..., None] + 1e-6
        o = num / den
        return (lambda x, *d: x.transpose(*d))(o, 0, 2, 1, 3).reshape(B, S, D) @ wo

    def _B_ref(x, w_gate, w_up, w_down):
        g = _silu(x @ w_gate)
        u = x @ w_up
        return (g * u) @ w_down

    x = A_x
    g = _sigmoid((x * gate_w).sum(-1, keepdims=True))
    a = _A_ref(x, A_wqkv, A_wo)
    b = _B_ref(x, B_w_gate, B_w_up, B_w_down)
    return g * a + (1 - g) * b
```

```python
import jax
import jax.numpy as jnp
from jax import lax
import jax.experimental.pallas as pl
import jax.experimental.pallas.tpu as pltpu

S, D, F, H = 2048, 512, 1792, 32
DH = D // H
HALF = D // 2
LANES = 128
SUBL = 8
NT = D // LANES
HB = LANES // DH
BF = jnp.bfloat16
F32 = jnp.float32

X1, X2, X3 = 256, 512, 1280
QT = 512
TM = 1024
SUB = 512
TAIL = (256, 192, 64)


def _phi(t):
    return jnp.where(t > 0, t + 1.0, jnp.exp(t)) + 1e-6


def _dot(a, b):
    return jnp.dot(a, b, preferred_element_type=F32)


def _dot_tn(a, b):
    return lax.dot_general(a, b, (((0,), (0,)), ((), ())), preferred_element_type=F32)


def _slab_row(h, d):
    return (d // SUBL) * (H * SUBL) + h * SUBL + d % SUBL


def _slab_groups(c0, c1):
    return [(c - c0, _slab_row(c // DH, c % DH)) for c in range(c0, c1, SUBL)]


def _slab_put(ref, j, val):
    for o, r in _slab_groups(0, D):
        ref[j, r:r + SUBL, :] = val[o:o + SUBL, :]


def _slab_get(ref, j, h0, nh):
    return jnp.concatenate(
        [ref[j, pl.ds(_slab_row(h0, d), nh, stride=SUBL), :] for d in range(DH)], axis=0)


def _kernel(x_hbm, wqkv_hbm, wo_hbm, wg_hbm, wu_hbm, wd_hbm, gw_hbm, out_hbm,
            x_v, wq_v, wk_v, wv_v, wo_v, wg_v, wu_v, wd_v, gw_v, out_v,
            g_acc, z_acc, m_v, wt_f32, zc_f32, wqp_v, pq_v, zp_v, sem):
    copy = pltpu.make_async_copy

    def xcopy(a, b, s):
        return copy(x_hbm.at[pl.ds(a, b - a)], x_v.at[pl.ds(a, b - a)], sem.at[s])

    grp1 = [xcopy(0, X1, 0),
            copy(wqkv_hbm.at[:, pl.ds(D, HALF)], wk_v.at[:, pl.ds(0, HALF)], sem.at[0])]
    grp2 = [copy(wqkv_hbm.at[:, pl.ds(D + HALF, HALF)], wk_v.at[:, pl.ds(HALF, HALF)], sem.at[1]),
            xcopy(X1, X2, 1)]
    grp3 = [xcopy(X2, X3, 0),
            copy(wqkv_hbm.at[:, pl.ds(0, D)], wq_v, sem.at[0])]
    grp4 = [xcopy(X3, S, 1),
            copy(wqkv_hbm.at[:, pl.ds(2 * D, D)], wv_v, sem.at[1]),
            copy(wo_hbm, wo_v, sem.at[1]),
            copy(gw_hbm, gw_v, sem.at[1])]
    grp5 = [copy(wg_hbm, wg_v, sem.at[0]),
            copy(wu_hbm, wu_v, sem.at[0]),
            copy(wd_hbm, wd_v, sem.at[0])]

    def start(grp):
        for c in grp:
            c.start()

    def wait(grp):
        for c in grp:
            c.wait()

    def ocopy(r, n):
        return copy(out_v.at[pl.ds(r, n)], out_hbm.at[pl.ds(r, n)], sem.at[1])

    def k_stage(a, b, c0, c1, first):
        pk = _phi(_dot(x_v[a:b, :], wk_v[:, c0:c1]))
        zs = jnp.sum(pk.reshape((b - a) // SUBL, SUBL, c1 - c0), axis=0)
        if first:
            z_acc[:, c0:c1] = zs
        else:
            z_acc[:, c0:c1] += zs
        return pk.astype(BF)

    def g_stage(pk, a, b, c0, c1, first):
        gp = _dot_tn(pk, x_v[a:b, :])
        for o, r in _slab_groups(c0, c1):
            for c in range(NT):
                blk = gp[o:o + SUBL, c * LANES:(c + 1) * LANES]
                if first:
                    g_acc[c, r:r + SUBL, :] = blk
                else:
                    g_acc[c, r:r + SUBL, :] += blk

    def key_stats(*jobs):
        pks = [k_stage(*job) for job in jobs]
        for pk, job in zip(pks, jobs):
            g_stage(pk, *job)

    def q_tile(a):
        pq_v[a:a + QT, :] = _phi(_dot(x_v[a:a + QT, :], wqp_v[...]))

    def attention_stats():
        wait(grp1)
        start(grp3)
        key_stats((0, X1, 0, LANES, True), (0, X1, LANES, HALF, True))

        wait(grp2)
        start(grp4)
        key_stats((0, X1, HALF, D, True), (X1, X2, 0, HALF, False), (X1, X2, HALF, D, False))

        wait(grp3)
        start(grp5)
        for j in range(NT):
            rows = slice(j * LANES, (j + 1) * LANES)
            _slab_put(wt_f32, j, wq_v[rows, :].T.astype(F32))
            wqp_v[rows, :] = _slab_get(wt_f32, j, 0, H).astype(BF).T
        key_stats((X2, X3, 0, D, False))

        wait(grp4)
        key_stats((X3, S, 0, D, False))

        z = jnp.sum(z_acc[...], axis=0, keepdims=True)
        _slab_put(zc_f32, 0, jnp.broadcast_to(z, (LANES, D)).T)
        zp_v[...] = _slab_get(zc_f32, 0, 0, H).T[0:SUBL, :]

        row_head = lax.broadcasted_iota(jnp.int32, (LANES, LANES), 0) % HB
        col_head = lax.broadcasted_iota(jnp.int32, (LANES, LANES), 1) // DH
        same_head = row_head == col_head
        kvs = []
        for j in range(NT):
            gj = jnp.concatenate([_slab_get(g_acc, c, j * HB, HB) for c in range(NT)], axis=1)
            kv = _dot(gj.astype(BF), wv_v[:, j * LANES:(j + 1) * LANES])
            kvs.append(jnp.where(same_head, kv, 0.0).astype(BF))
        q_tile(0)
        for j in range(NT):
            mj = _dot(kvs[j], wo_v[j * LANES:(j + 1) * LANES, :])
            for d in range(DH):
                r = d * H + j * HB
                m_v[r:r + HB, :] = mj[d * HB:(d + 1) * HB, :].astype(BF)
        for a in range(QT, S, QT):
            q_tile(a)

        wait(grp5)

    def normalized_q(r, n):
        pq = pq_v[pl.ds(r, n), :]
        t = pq * zp_v[0:1, :]
        t = (t[:, 0:128] + t[:, 128:256]) + (t[:, 256:384] + t[:, 384:512])
        t = t + pltpu.roll(t, 2 * H, 1)
        den = t + pltpu.roll(t, H, 1) + 1e-6
        inv = 1.0 / den
        return (pq * jnp.concatenate([inv] * NT, axis=1)).astype(BF)

    def mix_rows(i):
        for s0 in range(0, TM, SUB):
            r = pl.multiple_of(i * TM + s0, SUB)
            xt = x_v[pl.ds(r, SUB), :]
            gw = gw_v[...].astype(F32).reshape(1, D)
            logit = jnp.sum(xt.astype(F32) * gw, axis=-1, keepdims=True)
            gate = 0.5 * jnp.tanh(0.5 * logit) + 0.5
            hg = 0.5 * _dot(xt, wg_v[...])
            up = _dot(xt, wu_v[...])
            act = ((hg * jnp.tanh(hg) + hg) * up).astype(BF)
            o = 0
            for n in (TAIL if s0 + SUB == TM else (SUB,)):
                rr = pl.multiple_of(r + o, 64)
                a = _dot(normalized_q(rr, n), m_v[...])
                b = _dot(act[o:o + n, :], wd_v[...])
                out_v[pl.ds(rr, n), :] = (b + gate[o:o + n] * (a - b)).astype(BF)
                ocopy(rr, n).start()
                o += n

    start(grp1)
    start(grp2)

    def step(i, carry):
        @pl.when(i == 0)
        def _():
            attention_stats()

        @pl.when(i > 0)
        def _():
            mix_rows(i - 1)

        return carry

    lax.fori_loop(0, S // TM + 1, step, 0)
    ocopy(0, S).wait()


@jax.jit
def pallas_gated_mix__linear_attn_block__swiglu_ffn__prompt_kernel(
    A_x: jax.Array,
    A_wqkv: jax.Array,
    A_wo: jax.Array,
    B_x: jax.Array,
    B_w_gate: jax.Array,
    B_w_up: jax.Array,
    B_w_down: jax.Array,
    gate_w: jax.Array,
):
    del B_x
    hbm = pl.BlockSpec(memory_space=pl.ANY)
    vmem = pltpu.VMEM
    out = pl.pallas_call(
        _kernel,
        out_shape=jax.ShapeDtypeStruct((S, D), BF),
        in_specs=[hbm] * 7,
        out_specs=hbm,
        scratch_shapes=[
            vmem((S, D), BF),
            vmem((D, D), BF), vmem((D, D), BF), vmem((D, D), BF),
            vmem((D, D), BF),
            vmem((D, F), BF), vmem((D, F), BF), vmem((F, D), BF),
            vmem((D,), BF),
            vmem((S, D), BF),
            vmem((NT, D, LANES), F32),
            vmem((SUBL, D), F32),
            vmem((D, D), BF),
            vmem((NT, D, LANES), F32),
            vmem((1, D, LANES), F32),
            vmem((D, D), BF),
            vmem((S, D), F32),
            vmem((SUBL, D), F32),
            pltpu.SemaphoreType.DMA((2,)),
        ],
        compiler_params=pltpu.CompilerParams(vmem_limit_bytes=100 * 1024 * 1024),
        name="gated_mix",
    )(A_x.reshape(S, D), A_wqkv, A_wo, B_w_gate, B_w_up, B_w_down, gate_w)
    return out.reshape(1, S, D)
```

```python
import jax
import jax.numpy as jnp
from jax import lax
import jax.experimental.pallas as pl
import jax.experimental.pallas.tpu as pltpu

S, D, F, H = 2048, 512, 1792, 32
DH = D // H
HALF = D // 2
LANES = 128
SUBL = 8
NT = D // LANES
HB = LANES // DH
BF = jnp.bfloat16
F32 = jnp.float32

X1, X2, X3, X4 = 128, 512, 896, 1536
QT = 512
TM = 1024
SUB = 512
TAIL = (256, 192, 64)


def _phi(t):
    return jnp.where(t > 0, t + 1.0, jnp.exp(t)) + 1e-6


def _dot(a, b):
    return jnp.dot(a, b, preferred_element_type=F32)


def _dot_tn(a, b):
    return lax.dot_general(a, b, (((0,), (0,)), ((), ())), preferred_element_type=F32)


def _slab_row(h, d):
    return (d // SUBL) * (H * SUBL) + h * SUBL + d % SUBL


def _slab_parts(val, h0):
    nh, w = val.shape[0] // DH, val.shape[1]
    v = val.reshape(nh, DH // SUBL, SUBL, w)
    return [(_slab_row(h0, g * SUBL), v[:, g].reshape(nh * SUBL, w)) for g in range(DH // SUBL)]


def _slab_put(ref, j, val):
    for r, part in _slab_parts(val, 0):
        ref[j, r:r + part.shape[0], :] = part


def _slab_get(ref, j, h0, nh):
    return jnp.concatenate(
        [ref[j, pl.ds(_slab_row(h0, d), nh, stride=SUBL), :] for d in range(DH)], axis=0)


def _kernel(x_hbm, wqkv_hbm, wo_hbm, wg_hbm, wu_hbm, wd_hbm, gw_hbm, out_hbm,
            x_v, wq_v, wk_v, wv_v, wo_v, wg_v, wu_v, wd_v, gw_v, out_v,
            g_acc, z_acc, m_v, wt_f32, zc_f32, wqp_v, pq_v, zp_v, sem):
    copy = pltpu.make_async_copy

    def xcopy(a, b, s):
        return copy(x_hbm.at[pl.ds(a, b - a)], x_v.at[pl.ds(a, b - a)], sem.at[s])

    grp1 = [xcopy(0, X1, 0),
            copy(wqkv_hbm.at[:, pl.ds(D, HALF)], wk_v.at[:, pl.ds(0, HALF)], sem.at[0])]
    grp2 = [xcopy(X1, X2, 1)]
    grp3 = [copy(wqkv_hbm.at[:, pl.ds(D + HALF, HALF)], wk_v.at[:, pl.ds(HALF, HALF)], sem.at[0]),
            xcopy(X2, X3, 0)]
    grp4 = [xcopy(X3, S, 1),
            copy(wqkv_hbm.at[:, pl.ds(0, D)], wq_v, sem.at[1]),
            copy(wqkv_hbm.at[:, pl.ds(2 * D, D)], wv_v, sem.at[1]),
            copy(wo_hbm, wo_v, sem.at[1]),
            copy(gw_hbm, gw_v, sem.at[1])]
    grp5 = [copy(wg_hbm, wg_v, sem.at[0]),
            copy(wu_hbm, wu_v, sem.at[0]),
            copy(wd_hbm, wd_v, sem.at[0])]

    def start(grp):
        for c in grp:
            c.start()

    def wait(grp):
        for c in grp:
            c.wait()

    def ocopy(r, n):
        return copy(out_v.at[pl.ds(r, n)], out_hbm.at[pl.ds(r, n)], sem.at[1])

    def k_stage(a, b, c0, c1, first):
        pk = _phi(_dot(x_v[a:b, :], wk_v[:, c0:c1]))
        zs = jnp.sum(pk.reshape((b - a) // SUBL, SUBL, c1 - c0), axis=0)
        if first:
            z_acc[:, c0:c1] = zs
        else:
            z_acc[:, c0:c1] += zs
        return pk.astype(BF)

    def g_stage(pk, a, b, c0, c1, first):
        gp = _dot_tn(pk, x_v[a:b, :])
        for r, part in _slab_parts(gp, c0 // DH):
            rows = slice(r, r + part.shape[0])
            for c in range(NT):
                blk = part[:, c * LANES:(c + 1) * LANES]
                if first:
                    g_acc[c, rows, :] = blk
                else:
                    g_acc[c, rows, :] += blk

    def key_stats(*jobs):
        pks = [k_stage(*job) for job in jobs]
        for pk, job in zip(pks, jobs):
            g_stage(pk, *job)

    def q_tile(a):
        pq_v[a:a + QT, :] = _phi(_dot(x_v[a:a + QT, :], wqp_v[...]))

    def attention_stats():
        wait(grp1)
        start(grp3)
        key_stats((0, X1, 0, LANES, True), (0, X1, LANES, HALF, True))

        wait(grp2)
        start(grp4)
        key_stats((X1, X2, 0, LANES, False), (X1, X2, LANES, HALF, False))

        wait(grp3)
        start(grp5)
        key_stats((0, X2, HALF, D, True), (X2, X3, 0, HALF, False), (X2, X3, HALF, D, False))

        wait(grp4)
        for j in range(NT):
            rows = slice(j * LANES, (j + 1) * LANES)
            _slab_put(wt_f32, j, wq_v[rows, :].T.astype(F32))
            wqp_v[rows, :] = _slab_get(wt_f32, j, 0, H).astype(BF).T
        key_stats((X3, X4, 0, D, False))
        key_stats((X4, S, 0, D, False))

        z = jnp.sum(z_acc[...], axis=0, keepdims=True)
        _slab_put(zc_f32, 0, jnp.broadcast_to(z, (LANES, D)).T)
        zp_v[...] = _slab_get(zc_f32, 0, 0, H).T[0:SUBL, :]

        row_head = lax.broadcasted_iota(jnp.int32, (LANES, LANES), 0) % HB
        col_head = lax.broadcasted_iota(jnp.int32, (LANES, LANES), 1) // DH
        same_head = row_head == col_head
        kvs = []
        for j in range(NT):
            gj = jnp.concatenate([_slab_get(g_acc, c, j * HB, HB) for c in range(NT)], axis=1)
            kv = _dot(gj.astype(BF), wv_v[:, j * LANES:(j + 1) * LANES])
            kvs.append(jnp.where(same_head, kv, 0.0).astype(BF))
        q_tile(0)
        for j in range(NT):
            mj = _dot(kvs[j], wo_v[j * LANES:(j + 1) * LANES, :])
            for d in range(DH):
                r = d * H + j * HB
                m_v[r:r + HB, :] = mj[d * HB:(d + 1) * HB, :].astype(BF)
        for a in range(QT, S, QT):
            q_tile(a)

        wait(grp5)

    def normalized_q(r, n):
        pq = pq_v[pl.ds(r, n), :]
        t = pq * zp_v[0:1, :]
        t = (t[:, 0:128] + t[:, 128:256]) + (t[:, 256:384] + t[:, 384:512])
        t = t + pltpu.roll(t, 2 * H, 1)
        den = t + pltpu.roll(t, H, 1) + 1e-6
        inv = 1.0 / den
        return (pq * jnp.concatenate([inv] * NT, axis=1)).astype(BF)

    def mix_rows(i):
        for s0 in range(0, TM, SUB):
            r = pl.multiple_of(i * TM + s0, SUB)
            xt = x_v[pl.ds(r, SUB), :]
            gw = gw_v[...].astype(F32).reshape(1, D)
            logit = jnp.sum(xt.astype(F32) * gw, axis=-1, keepdims=True)
            gate = 0.5 * jnp.tanh(0.5 * logit) + 0.5
            hg = 0.5 * _dot(xt, wg_v[...])
            up = _dot(xt, wu_v[...])
            act = ((hg * jnp.tanh(hg) + hg) * up).astype(BF)
            o = 0
            for n in (TAIL if s0 + SUB == TM else (SUB,)):
                rr = pl.multiple_of(r + o, 64)
                a = _dot(normalized_q(rr, n), m_v[...])
                b = _dot(act[o:o + n, :], wd_v[...])
                out_v[pl.ds(rr, n), :] = (b + gate[o:o + n] * (a - b)).astype(BF)
                ocopy(rr, n).start()
                o += n

    start(grp1)
    start(grp2)

    def step(i, carry):
        @pl.when(i == 0)
        def _():
            attention_stats()

        @pl.when(i > 0)
        def _():
            mix_rows(i - 1)

        return carry

    lax.fori_loop(0, S // TM + 1, step, 0)
    ocopy(0, S).wait()


@jax.jit
def pallas_gated_mix__linear_attn_block__swiglu_ffn__prompt_kernel(
    A_x: jax.Array,
    A_wqkv: jax.Array,
    A_wo: jax.Array,
    B_x: jax.Array,
    B_w_gate: jax.Array,
    B_w_up: jax.Array,
    B_w_down: jax.Array,
    gate_w: jax.Array,
):
    del B_x
    hbm = pl.BlockSpec(memory_space=pl.ANY)
    vmem = pltpu.VMEM
    out = pl.pallas_call(
        _kernel,
        out_shape=jax.ShapeDtypeStruct((S, D), BF),
        in_specs=[hbm] * 7,
        out_specs=hbm,
        scratch_shapes=[
            vmem((S, D), BF),
            vmem((D, D), BF), vmem((D, D), BF), vmem((D, D), BF),
            vmem((D, D), BF),
            vmem((D, F), BF), vmem((D, F), BF), vmem((F, D), BF),
            vmem((D,), BF),
            vmem((S, D), BF),
            vmem((NT, D, LANES), F32),
            vmem((SUBL, D), F32),
            vmem((D, D), BF),
            vmem((NT, D, LANES), F32),
            vmem((1, D, LANES), F32),
            vmem((D, D), BF),
            vmem((S, D), F32),
            vmem((SUBL, D), F32),
            pltpu.SemaphoreType.DMA((2,)),
        ],
        compiler_params=pltpu.CompilerParams(vmem_limit_bytes=100 * 1024 * 1024),
        name="gated_mix",
    )(A_x.reshape(S, D), A_wqkv, A_wo, B_w_gate, B_w_up, B_w_down, gate_w)
    return out.reshape(1, S, D)
```

```python
import jax
import jax.numpy as jnp
from jax import lax
import jax.experimental.pallas as pl
import jax.experimental.pallas.tpu as pltpu

S, D, F, H = 2048, 512, 1792, 32
DH = D // H
HALF = D // 2
LANES = 128
SUBL = 8
NT = D // LANES
HB = LANES // DH
BF = jnp.bfloat16
F32 = jnp.float32
LOG2E = 1.4426950408889634

X1, X2, X3, X4 = 128, 512, 896, 1536
QPRE = 256
TM = 1024
SUB = 512
TAIL = (256, 192, 64)


def _phi(t):
    return jnp.where(t > 0, t + 1.0, jnp.exp(t)) + 1e-6


def _dot(a, b):
    return jnp.dot(a, b, preferred_element_type=F32)


def _dot_tn(a, b):
    return lax.dot_general(a, b, (((0,), (0,)), ((), ())), preferred_element_type=F32)


def _slab_row(h, d):
    return (d // SUBL) * (H * SUBL) + h * SUBL + d % SUBL


def _slab_parts(val, h0):
    nh, w = val.shape[0] // DH, val.shape[1]
    v = val.reshape(nh, DH // SUBL, SUBL, w)
    return [(_slab_row(h0, g * SUBL), v[:, g].reshape(nh * SUBL, w)) for g in range(DH // SUBL)]


def _slab_put(ref, j, val):
    for r, part in _slab_parts(val, 0):
        ref[j, r:r + part.shape[0], :] = part


def _slab_get(ref, j, h0, nh):
    return jnp.concatenate(
        [ref[j, pl.ds(_slab_row(h0, d), nh, stride=SUBL), :] for d in range(DH)], axis=0)


def _kernel(x_hbm, wqkv_hbm, wo_hbm, wg_hbm, wu_hbm, wd_hbm, gw_hbm, out_hbm,
            x_v, wq_v, wk_v, wv_v, wo_v, wg_v, wu_v, wd_v, gw_v, out_v,
            g_acc, z_acc, m_v, wt_f32, zc_f32, wqp_v, pq_v, zp_v, sem):
    copy = pltpu.make_async_copy

    def xcopy(a, b, s):
        return copy(x_hbm.at[pl.ds(a, b - a)], x_v.at[pl.ds(a, b - a)], sem.at[s])

    grp1 = [copy(wqkv_hbm.at[:, pl.ds(D, HALF)], wk_v.at[:, pl.ds(0, HALF)], sem.at[0]),
            xcopy(0, X1, 0)]
    grp2 = [xcopy(X1, X2, 1)]
    grp3 = [copy(wqkv_hbm.at[:, pl.ds(D + HALF, HALF)], wk_v.at[:, pl.ds(HALF, HALF)], sem.at[0]),
            xcopy(X2, X3, 0)]
    grp4 = [xcopy(X3, S, 1),
            copy(wqkv_hbm.at[:, pl.ds(0, D)], wq_v, sem.at[1]),
            copy(wqkv_hbm.at[:, pl.ds(2 * D, D)], wv_v, sem.at[1]),
            copy(wo_hbm, wo_v, sem.at[1]),
            copy(gw_hbm, gw_v, sem.at[1])]
    grp5 = [copy(wg_hbm, wg_v, sem.at[0]),
            copy(wu_hbm, wu_v, sem.at[0]),
            copy(wd_hbm, wd_v, sem.at[0])]

    def start(grp):
        for c in grp:
            c.start()

    def wait(grp):
        for c in grp:
            c.wait()

    def ocopy(r, n):
        return copy(out_v.at[pl.ds(r, n)], out_hbm.at[pl.ds(r, n)], sem.at[1])

    def k_stage(a, b, c0, c1, first):
        pk = _phi(_dot(x_v[a:b, :], wk_v[:, c0:c1]))
        zs = jnp.sum(pk.reshape((b - a) // SUBL, SUBL, c1 - c0), axis=0)
        if first:
            z_acc[:, c0:c1] = zs
        else:
            z_acc[:, c0:c1] += zs
        return pk.astype(BF)

    def g_stage(pk, a, b, c0, c1, first):
        gp = _dot_tn(pk, x_v[a:b, :])
        for r, part in _slab_parts(gp, c0 // DH):
            rows = slice(r, r + part.shape[0])
            for c in range(NT):
                blk = part[:, c * LANES:(c + 1) * LANES]
                if first:
                    g_acc[c, rows, :] = blk
                else:
                    g_acc[c, rows, :] += blk

    def key_stats(*jobs):
        pks = [k_stage(*job) for job in jobs]
        for pk, job in zip(pks, jobs):
            g_stage(pk, *job)

    def q_rows(a, n):
        pq_v[pl.ds(a, n), :] = _phi(_dot(x_v[pl.ds(a, n), :], wqp_v[...]))

    def attention_stats():
        wait(grp1)
        start(grp3)
        key_stats((0, X1, 0, LANES, True), (0, X1, LANES, HALF, True))

        wait(grp2)
        start(grp4)
        key_stats((X1, X2, 0, LANES, False), (X1, X2, LANES, HALF, False))

        wait(grp3)
        start(grp5)
        key_stats((0, X2, HALF, D, True), (X2, X3, 0, HALF, False), (X2, X3, HALF, D, False))

        wait(grp4)
        for j in range(NT):
            rows = slice(j * LANES, (j + 1) * LANES)
            _slab_put(wt_f32, j, wq_v[rows, :].T.astype(F32))
            wqp_v[rows, :] = _slab_get(wt_f32, j, 0, H).astype(BF).T
        key_stats((X3, X4, 0, D, False))
        key_stats((X4, S, 0, D, False))

        z = jnp.sum(z_acc[...], axis=0, keepdims=True)
        _slab_put(zc_f32, 0, jnp.broadcast_to(z, (LANES, D)).T)
        zp_v[...] = _slab_get(zc_f32, 0, 0, H).T[0:SUBL, :]

        row_head = lax.broadcasted_iota(jnp.int32, (LANES, LANES), 0) % HB
        col_head = lax.broadcasted_iota(jnp.int32, (LANES, LANES), 1) // DH
        same_head = row_head == col_head
        kvs = []
        for j in range(NT):
            gj = jnp.concatenate([_slab_get(g_acc, c, j * HB, HB) for c in range(NT)], axis=1)
            kv = _dot(gj.astype(BF), wv_v[:, j * LANES:(j + 1) * LANES])
            kvs.append(jnp.where(same_head, kv, 0.0).astype(BF))
        for a in range(0, S, TM):
            q_rows(a, QPRE)
        for j in range(NT):
            mj = _dot(kvs[j], wo_v[j * LANES:(j + 1) * LANES, :])
            for d in range(DH):
                r = d * H + j * HB
                m_v[r:r + HB, :] = mj[d * HB:(d + 1) * HB, :].astype(BF)

        wait(grp5)

    def normalized_q(r, n):
        pq = pq_v[pl.ds(r, n), :]
        t = pq * zp_v[0:1, :]
        t = (t[:, 0:128] + t[:, 128:256]) + (t[:, 256:384] + t[:, 384:512])
        t = t + pltpu.roll(t, 2 * H, 1)
        den = t + pltpu.roll(t, H, 1) + 1e-6
        inv = pl.reciprocal(den, approx=True)
        return (pq * jnp.concatenate([inv] * NT, axis=1)).astype(BF)

    def mix_rows(i):
        q_rows(pl.multiple_of(i * TM + QPRE, QPRE), TM - QPRE)
        for s0 in range(0, TM, SUB):
            r = pl.multiple_of(i * TM + s0, SUB)
            xt = x_v[pl.ds(r, SUB), :]
            gw = gw_v[...].astype(F32).reshape(1, D)
            logit = jnp.sum(xt.astype(F32) * gw, axis=-1, keepdims=True)
            gate = 1.0 / (1.0 + jnp.exp(-logit))
            pre = _dot(xt, wg_v[...])
            up = _dot(xt, wu_v[...])
            sig = pl.reciprocal(1.0 + jnp.exp2(pre * -LOG2E), approx=True)
            act = (pre * sig * up).astype(BF)
            o = 0
            for n in (TAIL if s0 + SUB == TM else (SUB,)):
                rr = pl.multiple_of(r + o, 64)
                a = _dot(normalized_q(rr, n), m_v[...])
                b = _dot(act[o:o + n, :], wd_v[...])
                out_v[pl.ds(rr, n), :] = (gate[o:o + n] * a + (1.0 - gate[o:o + n]) * b).astype(BF)
                ocopy(rr, n).start()
                o += n

    start(grp1)
    start(grp2)

    def step(i, carry):
        @pl.when(i == 0)
        def _():
            attention_stats()

        @pl.when(i > 0)
        def _():
            mix_rows(i - 1)

        return carry

    lax.fori_loop(0, S // TM + 1, step, 0)
    ocopy(0, S).wait()


@jax.jit
def pallas_gated_mix__linear_attn_block__swiglu_ffn__prompt_kernel(
    A_x: jax.Array,
    A_wqkv: jax.Array,
    A_wo: jax.Array,
    B_x: jax.Array,
    B_w_gate: jax.Array,
    B_w_up: jax.Array,
    B_w_down: jax.Array,
    gate_w: jax.Array,
):
    del B_x
    hbm = pl.BlockSpec(memory_space=pl.ANY)
    vmem = pltpu.VMEM
    out = pl.pallas_call(
        _kernel,
        out_shape=jax.ShapeDtypeStruct((S, D), BF),
        in_specs=[hbm] * 7,
        out_specs=hbm,
        scratch_shapes=[
            vmem((S, D), BF),
            vmem((D, D), BF), vmem((D, D), BF), vmem((D, D), BF),
            vmem((D, D), BF),
            vmem((D, F), BF), vmem((D, F), BF), vmem((F, D), BF),
            vmem((D,), BF),
            vmem((S, D), BF),
            vmem((NT, D, LANES), F32),
            vmem((SUBL, D), F32),
            vmem((D, D), BF),
            vmem((NT, D, LANES), F32),
            vmem((1, D, LANES), F32),
            vmem((D, D), BF),
            vmem((S, D), F32),
            vmem((SUBL, D), F32),
            pltpu.SemaphoreType.DMA((2,)),
        ],
        compiler_params=pltpu.CompilerParams(vmem_limit_bytes=64 * 1024 * 1024),
        name="gated_mix",
    )(A_x.reshape(S, D), A_wqkv, A_wo, B_w_gate, B_w_up, B_w_down, gate_w)
    return out.reshape(1, S, D)
```

```python
import jax
import jax.numpy as jnp
from jax import lax
import jax.experimental.pallas as pl
import jax.experimental.pallas.tpu as pltpu

S, D, F, H = 2048, 512, 1792, 32
DH = D // H
HALF = D // 2
LANES = 128
SUBL = 8
NT = D // LANES
HB = LANES // DH
BF = jnp.bfloat16
F32 = jnp.float32
LOG2E = 1.4426950408889634

X1, X2, X3, X4 = 128, 512, 896, 1536
QPRE = 256
TM = 1024
SUB = 512
TAIL = (320, 128, 64)
LAST_COLS = ((0, 384), (384, D))


def _phi(t):
    return jnp.where(t > 0, t + 1.0, jnp.exp(t)) + 1e-6


def _dot(a, b):
    return jnp.dot(a, b, preferred_element_type=F32)


def _dot_tn(a, b):
    return lax.dot_general(a, b, (((0,), (0,)), ((), ())), preferred_element_type=F32)


def _slab_row(h, d):
    return (d // SUBL) * (H * SUBL) + h * SUBL + d % SUBL


def _slab_parts(val, h0):
    nh, w = val.shape[0] // DH, val.shape[1]
    v = val.reshape(nh, DH // SUBL, SUBL, w)
    return [(_slab_row(h0, g * SUBL), v[:, g].reshape(nh * SUBL, w)) for g in range(DH // SUBL)]


def _slab_put(ref, j, val):
    for r, part in _slab_parts(val, 0):
        ref[j, r:r + part.shape[0], :] = part


def _slab_get(ref, j, h0, nh):
    return jnp.concatenate(
        [ref[j, pl.ds(_slab_row(h0, d), nh, stride=SUBL), :] for d in range(DH)], axis=0)


def _kernel(x_hbm, wqkv_hbm, wo_hbm, wg_hbm, wu_hbm, wd_hbm, gw_hbm, out_hbm,
            x_v, wq_v, wk_v, wv_v, wo_v, wg_v, wu_v, wd_v, gw_v, out_v,
            g_acc, z_acc, m_v, wt_f32, zc_f32, wqp_v, pq_v, zp_v, sem):
    copy = pltpu.make_async_copy

    def xcopy(a, b, s):
        return copy(x_hbm.at[pl.ds(a, b - a)], x_v.at[pl.ds(a, b - a)], sem.at[s])

    grp1 = [copy(wqkv_hbm.at[:, pl.ds(D, HALF)], wk_v.at[:, pl.ds(0, HALF)], sem.at[0]),
            xcopy(0, X1, 0)]
    grp2 = [xcopy(X1, X2, 1)]
    grp3 = [copy(wqkv_hbm.at[:, pl.ds(D + HALF, HALF)], wk_v.at[:, pl.ds(HALF, HALF)], sem.at[0]),
            xcopy(X2, X3, 0)]
    grp4 = [xcopy(X3, S, 1),
            copy(wqkv_hbm.at[:, pl.ds(0, D)], wq_v, sem.at[1]),
            copy(wqkv_hbm.at[:, pl.ds(2 * D, D)], wv_v, sem.at[1]),
            copy(wo_hbm, wo_v, sem.at[1]),
            copy(gw_hbm, gw_v, sem.at[1])]
    grp5 = [copy(wg_hbm, wg_v, sem.at[0]),
            copy(wu_hbm, wu_v, sem.at[0]),
            copy(wd_hbm, wd_v, sem.at[0])]

    def start(grp):
        for c in grp:
            c.start()

    def wait(grp):
        for c in grp:
            c.wait()

    def ocopy(r, n, c0, c1):
        rows, cols = pl.ds(r, n), pl.ds(c0, c1 - c0)
        return copy(out_v.at[rows, cols], out_hbm.at[rows, cols], sem.at[1])

    def k_stage(a, b, c0, c1, first):
        pk = _phi(_dot(x_v[a:b, :], wk_v[:, c0:c1]))
        zs = jnp.sum(pk.reshape((b - a) // SUBL, SUBL, c1 - c0), axis=0)
        if first:
            z_acc[:, c0:c1] = zs
        else:
            z_acc[:, c0:c1] += zs
        return pk.astype(BF)

    def g_stage(pk, a, b, c0, c1, first):
        gp = _dot_tn(pk, x_v[a:b, :])
        for r, part in _slab_parts(gp, c0 // DH):
            rows = slice(r, r + part.shape[0])
            for c in range(NT):
                blk = part[:, c * LANES:(c + 1) * LANES]
                if first:
                    g_acc[c, rows, :] = blk
                else:
                    g_acc[c, rows, :] += blk

    def key_stats(*jobs):
        pks = [k_stage(*job) for job in jobs]
        for pk, job in zip(pks, jobs):
            g_stage(pk, *job)

    def q_rows(a, n):
        pq_v[pl.ds(a, n), :] = _phi(_dot(x_v[pl.ds(a, n), :], wqp_v[...]))

    def attention_stats():
        wait(grp1)
        start(grp3)
        key_stats((0, X1, 0, LANES, True), (0, X1, LANES, HALF, True))

        wait(grp2)
        start(grp4)
        key_stats((X1, X2, 0, LANES, False), (X1, X2, LANES, HALF, False))

        wait(grp3)
        start(grp5)
        key_stats((0, X2, HALF, D, True), (X2, X3, 0, HALF, False), (X2, X3, HALF, D, False))

        wait(grp4)
        for j in range(NT):
            rows = slice(j * LANES, (j + 1) * LANES)
            _slab_put(wt_f32, j, wq_v[rows, :].T.astype(F32))
            wqp_v[rows, :] = _slab_get(wt_f32, j, 0, H).astype(BF).T
        key_stats((X3, X4, 0, D, False))
        key_stats((X4, S, 0, D, False))

        z = jnp.sum(z_acc[...], axis=0, keepdims=True)
        _slab_put(zc_f32, 0, jnp.broadcast_to(z, (LANES, D)).T)
        zp_v[...] = _slab_get(zc_f32, 0, 0, H).T[0:SUBL, :]

        row_head = lax.broadcasted_iota(jnp.int32, (LANES, LANES), 0) % HB
        col_head = lax.broadcasted_iota(jnp.int32, (LANES, LANES), 1) // DH
        same_head = row_head == col_head
        kvs = []
        for j in range(NT):
            gj = jnp.concatenate([_slab_get(g_acc, c, j * HB, HB) for c in range(NT)], axis=1)
            kv = _dot(gj.astype(BF), wv_v[:, j * LANES:(j + 1) * LANES])
            kvs.append(jnp.where(same_head, kv, 0.0).astype(BF))
        for a in range(0, S, TM):
            q_rows(a, QPRE)
        for j in range(NT):
            mj = _dot(kvs[j], wo_v[j * LANES:(j + 1) * LANES, :])
            for d in range(DH):
                r = d * H + j * HB
                m_v[r:r + HB, :] = mj[d * HB:(d + 1) * HB, :].astype(BF)

        wait(grp5)

    def normalized_q(r, n):
        pq = pq_v[pl.ds(r, n), :]
        t = pq * zp_v[0:1, :]
        t = (t[:, 0:128] + t[:, 128:256]) + (t[:, 256:384] + t[:, 384:512])
        t = t + pltpu.roll(t, 2 * H, 1)
        den = t + pltpu.roll(t, H, 1) + 1e-6
        inv = pl.reciprocal(den, approx=True)
        return (pq * jnp.concatenate([inv] * NT, axis=1)).astype(BF)

    def mix_rows(i):
        q_rows(pl.multiple_of(i * TM + QPRE, QPRE), TM - QPRE)
        for s0 in range(0, TM, SUB):
            r = pl.multiple_of(i * TM + s0, SUB)
            xt = x_v[pl.ds(r, SUB), :]
            gw = gw_v[...].astype(F32).reshape(1, D)
            logit = jnp.sum(xt.astype(F32) * gw, axis=-1, keepdims=True)
            gate = 1.0 / (1.0 + jnp.exp(-logit))
            pre = _dot(xt, wg_v[...])
            up = _dot(xt, wu_v[...])
            sig = pl.reciprocal(1.0 + jnp.exp2(pre * -LOG2E), approx=True)
            act = (pre * sig * up).astype(BF)
            o = 0
            for n in (TAIL if s0 + SUB == TM else (SUB,)):
                rr = pl.multiple_of(r + o, 64)
                pqn = normalized_q(rr, n)
                g = gate[o:o + n]
                for c0, c1 in (LAST_COLS if s0 + o + n == TM else ((0, D),)):
                    a = _dot(pqn, m_v[:, c0:c1])
                    b = _dot(act[o:o + n, :], wd_v[:, c0:c1])
                    out_v[pl.ds(rr, n), c0:c1] = (g * a + (1.0 - g) * b).astype(BF)
                    ocopy(rr, n, c0, c1).start()
                o += n

    start(grp1)
    start(grp2)

    def step(i, carry):
        @pl.when(i == 0)
        def _():
            attention_stats()

        @pl.when(i > 0)
        def _():
            mix_rows(i - 1)

        return carry

    lax.fori_loop(0, S // TM + 1, step, 0)
    ocopy(0, S, 0, D).wait()


@jax.jit
def pallas_gated_mix__linear_attn_block__swiglu_ffn__prompt_kernel(
    A_x: jax.Array,
    A_wqkv: jax.Array,
    A_wo: jax.Array,
    B_x: jax.Array,
    B_w_gate: jax.Array,
    B_w_up: jax.Array,
    B_w_down: jax.Array,
    gate_w: jax.Array,
):
    del B_x
    hbm = pl.BlockSpec(memory_space=pl.ANY)
    vmem = pltpu.VMEM
    out = pl.pallas_call(
        _kernel,
        out_shape=jax.ShapeDtypeStruct((S, D), BF),
        in_specs=[hbm] * 7,
        out_specs=hbm,
        scratch_shapes=[
            vmem((S, D), BF),
            vmem((D, D), BF), vmem((D, D), BF), vmem((D, D), BF),
            vmem((D, D), BF),
            vmem((D, F), BF), vmem((D, F), BF), vmem((F, D), BF),
            vmem((D,), BF),
            vmem((S, D), BF),
            vmem((NT, D, LANES), F32),
            vmem((SUBL, D), F32),
            vmem((D, D), BF),
            vmem((NT, D, LANES), F32),
            vmem((1, D, LANES), F32),
            vmem((D, D), BF),
            vmem((S, D), F32),
            vmem((SUBL, D), F32),
            pltpu.SemaphoreType.DMA((2,)),
        ],
        compiler_params=pltpu.CompilerParams(vmem_limit_bytes=64 * 1024 * 1024),
        name="gated_mix",
    )(A_x.reshape(S, D), A_wqkv, A_wo, B_w_gate, B_w_up, B_w_down, gate_w)
    return out.reshape(1, S, D)
```

```python
import jax
import jax.numpy as jnp
from jax import lax
import jax.experimental.pallas as pl
import jax.experimental.pallas.tpu as pltpu

S, D, F, H = 2048, 512, 1792, 32
DH = D // H
HALF = D // 2
LANES = 128
SUBL = 8
NT = D // LANES
PITCH = H + SUBL
BF = jnp.bfloat16
F32 = jnp.float32
LOG2E = 1.4426950408889634

X1, X2, X3, X4 = 128, 512, 896, 1536
QPRE = 384
TM = 1024
SUB = 512
TAIL = (320, 128, 64)
LAST_COLS = ((0, 384), (384, D))


def _phi(t):
    return jnp.where(t > 0, t + 1.0, jnp.exp(t)) + 1e-6


def _dot(a, b):
    return jnp.dot(a, b, preferred_element_type=F32)


def _dot_tn(a, b):
    return lax.dot_general(a, b, (((0,), (0,)), ((), ())), preferred_element_type=F32)


def _tile(c):
    return slice(c * LANES, (c + 1) * LANES)


def _after(never, dep, val):
    return jnp.where(never, dep, val)


def _scatter(slab, c, val):
    for h in range(H):
        slab[c, pl.ds(h, DH, stride=PITCH), :] = val[h * DH:(h + 1) * DH, :]


def _heads(slab, c, h0, nh):
    return slab.reshape(slab.shape[0], DH, PITCH, LANES)[c, :, h0:h0 + nh, :]


def _kernel(x_hbm, wqkv_hbm, wo_hbm, wg_hbm, wu_hbm, wd_hbm, gw_hbm, out_hbm,
            x_v, wq_v, wk_v, wv_v, wo_v, wg_v, wu_v, wd_v, gw_v, out_v,
            g_acc, z_acc, wqp_v, pq_v, zp_v, m_v, wq_s, z_s, g_s, wv_s, wo_s, sem):
    copy = pltpu.make_async_copy

    def xcopy(a, b, s):
        return copy(x_hbm.at[pl.ds(a, b - a)], x_v.at[pl.ds(a, b - a)], sem.at[s])

    grp1 = [copy(wqkv_hbm.at[:, pl.ds(D, HALF)], wk_v.at[:, pl.ds(0, HALF)], sem.at[0]),
            xcopy(0, X1, 0)]
    grp2 = [xcopy(X1, X2, 1)]
    grp3 = [copy(wqkv_hbm.at[:, pl.ds(D + HALF, HALF)], wk_v.at[:, pl.ds(HALF, HALF)], sem.at[0]),
            xcopy(X2, X3, 0)]
    grp4 = [xcopy(X3, S, 1),
            copy(wqkv_hbm.at[:, pl.ds(0, D)], wq_v, sem.at[1]),
            copy(wqkv_hbm.at[:, pl.ds(2 * D, D)], wv_v, sem.at[1]),
            copy(wo_hbm, wo_v, sem.at[1]),
            copy(gw_hbm, gw_v, sem.at[1])]
    grp5 = [copy(wg_hbm, wg_v, sem.at[0]),
            copy(wu_hbm, wu_v, sem.at[0]),
            copy(wd_hbm, wd_v, sem.at[0])]

    def start(grp):
        for c in grp:
            c.start()

    def wait(grp):
        for c in grp:
            c.wait()

    def ocopy(r, n, c0, c1):
        rows, cols = pl.ds(r, n), pl.ds(c0, c1 - c0)
        return copy(out_v.at[rows, cols], out_hbm.at[rows, cols], sem.at[1])

    def phi_k(a, b, c0, c1, first):
        pk = _phi(_dot(x_v[a:b, :], wk_v[:, c0:c1]))
        zs = jnp.sum(pk.reshape((b - a) // SUBL, SUBL, c1 - c0), axis=0)
        if first:
            z_acc[:, c0:c1] = zs
        else:
            z_acc[:, c0:c1] += zs
        return pk.astype(BF)

    def key_stats(*jobs):
        pks = [phi_k(*job) for job in jobs]
        for pk, (a, b, c0, c1, first) in zip(pks, jobs):
            gp = _dot_tn(pk, x_v[a:b, :])
            if first:
                g_acc[c0:c1, :] = gp
            else:
                g_acc[c0:c1, :] += gp

    def phi_q(a, n):
        pq = _phi(_dot(x_v[pl.ds(a, n), :], wqp_v[...]))
        pq_v[pl.ds(a, n), :] = pq
        return pq

    def attention_stats(never):
        wait(grp1)
        start(grp3)
        key_stats((0, X1, 0, LANES, True), (0, X1, LANES, HALF, True))

        wait(grp2)
        start(grp4)
        key_stats((X1, X2, 0, LANES, False), (X1, X2, LANES, HALF, False))

        wait(grp3)
        start(grp5)
        key_stats((0, X2, HALF, D, True), (X2, X3, 0, HALF, False), (X2, X3, HALF, D, False))

        wait(grp4)
        wv_t = wv_v[...].T
        wq_t = wq_v[...].T
        pk = phi_k(X3, X4, 0, D, False)
        pk = jnp.concatenate([_after(never, wq_t, pk[0:D]), pk[D:]], axis=0)
        gp = _dot_tn(pk, x_v[X3:X4, :])
        g_acc[...] += gp
        g = g_acc[...] + _dot_tn(phi_k(X4, S, 0, D, False), x_v[X4:S, :])
        for c in range(NT):
            _scatter(g_s, c, g[:, _tile(c)])

        for c in range(NT):
            _scatter(wq_s, c, wq_t[:, _tile(c)].astype(F32))
            wqp_v[_tile(c), :] = _heads(wq_s, c, 0, H).reshape(D, LANES).astype(BF).T
        pq = jnp.concatenate([phi_q(a, QPRE) for a in range(0, S, TM)], axis=0)
        for c in range(NT):
            _scatter(wv_s, c, _after(never, pq[0:D, _tile(c)], wv_t[:, _tile(c)].astype(F32)))
            _scatter(wo_s, c, _after(never, gp[:, _tile(c)], wo_v[:, _tile(c)].astype(F32)))
        z = jnp.sum(z_acc[...], axis=0, keepdims=True)
        _scatter(z_s, 0, jnp.broadcast_to(z, (LANES, D)).T)
        zp_v[...] = _heads(z_s, 0, 0, H).reshape(D, LANES).T[0:SUBL, :]

        wait(grp5)

    def build_m(never):
        m = None
        for h0 in range(0, H, SUBL):
            for d in range(DH):
                r = d * PITCH + h0
                g = jnp.concatenate([g_s[c, r:r + SUBL, :] for c in range(NT)], axis=1)
                if m is not None:
                    g = _after(never, m, g)
                wv = jnp.concatenate([_heads(wv_s, c, h0, SUBL) for c in range(NT)], axis=2)
                kv = jnp.sum(g[None] * wv, axis=-1, keepdims=True)
                wo = jnp.concatenate([_heads(wo_s, c, h0, SUBL) for c in range(NT)], axis=2)
                m = jnp.sum(kv * wo, axis=0)
                m_v[d * H + h0:d * H + h0 + SUBL, :] = m.astype(BF)

    def normalized_q(r, n):
        pq = pq_v[pl.ds(r, n), :]
        t = pq * zp_v[0:1, :]
        t = (t[:, _tile(0)] + t[:, _tile(1)]) + (t[:, _tile(2)] + t[:, _tile(3)])
        t = t + pltpu.roll(t, 2 * H, 1)
        den = t + pltpu.roll(t, H, 1) + 1e-6
        inv = pl.reciprocal(den, approx=True)
        return (pq * jnp.concatenate([inv] * NT, axis=1)).astype(BF)

    def mix_rows(i, never):
        build_m(never)
        subs = []
        for s0 in range(0, TM, SUB):
            r = pl.multiple_of(i * TM + s0, SUB)
            xt = x_v[pl.ds(r, SUB), :]
            subs.append((s0, r, xt, _dot(xt, wg_v[...])))
        phi_q(pl.multiple_of(i * TM + QPRE, LANES), TM - QPRE)
        acts = []
        for s0, r, xt, pre in subs:
            gw = gw_v[...].astype(F32).reshape(1, D)
            logit = jnp.sum(xt.astype(F32) * gw, axis=-1, keepdims=True)
            gate = 1.0 / (1.0 + jnp.exp(-logit))
            up = _dot(xt, wu_v[...])
            sig = pl.reciprocal(1.0 + jnp.exp2(pre * -LOG2E), approx=True)
            acts.append((s0, r, gate, (pre * sig * up).astype(BF)))
        for s0, r, gate, act in acts:
            o = 0
            for n in (TAIL if s0 + SUB == TM else (SUB,)):
                rr = pl.multiple_of(r + o, 32)
                pqn = normalized_q(rr, n)
                g = gate[o:o + n]
                for c0, c1 in (LAST_COLS if s0 + o + n == TM else ((0, D),)):
                    a = _dot(pqn, m_v[:, c0:c1])
                    b = _dot(act[o:o + n, :], wd_v[:, c0:c1])
                    out_v[pl.ds(rr, n), c0:c1] = (g * a + (1.0 - g) * b).astype(BF)
                    ocopy(rr, n, c0, c1).start()
                o += n

    start(grp1)
    start(grp2)

    def step(i, carry):
        @pl.when(i == 0)
        def _():
            attention_stats(never=i > 0)

        @pl.when(i > 0)
        def _():
            mix_rows(i - 1, never=i - 1 < 0)

        return carry

    lax.fori_loop(0, S // TM + 1, step, 0)
    ocopy(0, S, 0, D).wait()


@jax.jit
def pallas_gated_mix__linear_attn_block__swiglu_ffn__prompt_kernel(
    A_x: jax.Array,
    A_wqkv: jax.Array,
    A_wo: jax.Array,
    B_x: jax.Array,
    B_w_gate: jax.Array,
    B_w_up: jax.Array,
    B_w_down: jax.Array,
    gate_w: jax.Array,
):
    del B_x
    hbm = pl.BlockSpec(memory_space=pl.ANY)
    vmem = pltpu.VMEM
    slab = vmem((NT, DH * PITCH, LANES), F32)
    out = pl.pallas_call(
        _kernel,
        out_shape=jax.ShapeDtypeStruct((S, D), BF),
        in_specs=[hbm] * 7,
        out_specs=hbm,
        scratch_shapes=[
            vmem((S, D), BF),
            vmem((D, D), BF), vmem((D, D), BF), vmem((D, D), BF),
            vmem((D, D), BF),
            vmem((D, F), BF), vmem((D, F), BF), vmem((F, D), BF),
            vmem((D,), BF),
            vmem((S, D), BF),
            vmem((D, D), F32),
            vmem((SUBL, D), F32),
            vmem((D, D), BF),
            vmem((S, D), F32),
            vmem((SUBL, D), F32),
            vmem((D, D), BF),
            slab,
            vmem((1, DH * PITCH, LANES), F32),
            slab, slab, slab,
            pltpu.SemaphoreType.DMA((2,)),
        ],
        compiler_params=pltpu.CompilerParams(vmem_limit_bytes=64 * 1024 * 1024),
        name="gated_mix",
    )(A_x.reshape(S, D), A_wqkv, A_wo, B_w_gate, B_w_up, B_w_down, gate_w)
    return out.reshape(1, S, D)
```

```python
import jax
import jax.numpy as jnp
from jax import lax
import jax.experimental.pallas as pl
import jax.experimental.pallas.tpu as pltpu

S, D, F, H = 2048, 512, 1792, 32
DH = D // H
HALF = D // 2
LANES = 128
SUBL = 8
NT = D // LANES
PITCH = H + SUBL
BF = jnp.bfloat16
F32 = jnp.float32
LOG2E = 1.4426950408889634

X1, X2, X3, X4 = 128, 512, 896, 1536
QPRE = 384
TM = 1024
SUB = 512
TAIL = (320, 128, 64)
LAST_COLS = ((0, 384), (384, D))


def _phi(t):
    return jnp.where(t > 0, t + 1.0, jnp.exp(t)) + 1e-6


def _dot(a, b):
    return jnp.dot(a, b, preferred_element_type=F32)


def _dot_tn(a, b):
    return lax.dot_general(a, b, (((0,), (0,)), ((), ())), preferred_element_type=F32)


def _tile(c):
    return slice(c * LANES, (c + 1) * LANES)


def _after(never, dep, val):
    return jnp.where(never, dep, val)


def _scatter(slab, c, val):
    for h in range(H):
        slab[c, pl.ds(h, DH, stride=PITCH), :] = val[h * DH:(h + 1) * DH, :]


def _heads(slab, c, h0, nh):
    return slab[c].reshape(DH, PITCH, LANES)[:, h0:h0 + nh, :]


def _kernel(x_hbm, wqkv_hbm, wo_hbm, wg_hbm, wu_hbm, wd_hbm, gw_hbm, out_hbm,
            x_v, wq_v, wk_v, wv_v, wo_v, wg_v, wu_v, wd_v, gw_v, out_v,
            g_acc, z_acc, wqp_v, pq_v, zp_v, m_v, wq_s, z_s, g_s, wv_s, wo_s, sem):
    copy = pltpu.make_async_copy

    def xcopy(a, b, s):
        return copy(x_hbm.at[pl.ds(a, b - a)], x_v.at[pl.ds(a, b - a)], sem.at[s])

    grp1 = [copy(wqkv_hbm.at[:, pl.ds(D, HALF)], wk_v.at[:, pl.ds(0, HALF)], sem.at[0]),
            xcopy(0, X1, 0)]
    grp2 = [xcopy(X1, X2, 1)]
    grp3 = [copy(wqkv_hbm.at[:, pl.ds(D + HALF, HALF)], wk_v.at[:, pl.ds(HALF, HALF)], sem.at[0]),
            xcopy(X2, X3, 0)]
    grp4 = [xcopy(X3, S, 1),
            copy(wqkv_hbm.at[:, pl.ds(0, D)], wq_v, sem.at[1]),
            copy(wqkv_hbm.at[:, pl.ds(2 * D, D)], wv_v, sem.at[1]),
            copy(wo_hbm, wo_v, sem.at[1]),
            copy(gw_hbm, gw_v, sem.at[1])]
    grp5 = [copy(wg_hbm, wg_v, sem.at[0]),
            copy(wu_hbm, wu_v, sem.at[0]),
            copy(wd_hbm, wd_v, sem.at[0])]

    def start(grp):
        for c in grp:
            c.start()

    def wait(grp):
        for c in grp:
            c.wait()

    def ocopy(r, n, c0, c1):
        rows, cols = pl.ds(r, n), pl.ds(c0, c1 - c0)
        return copy(out_v.at[rows, cols], out_hbm.at[rows, cols], sem.at[1])

    def phi_k(a, b, c0, c1, first):
        pk = _phi(_dot(x_v[a:b, :], wk_v[:, c0:c1]))
        zs = jnp.sum(pk.reshape((b - a) // SUBL, SUBL, c1 - c0), axis=0)
        if first:
            z_acc[:, c0:c1] = zs
        else:
            z_acc[:, c0:c1] += zs
        return pk.astype(BF)

    def key_stats(*jobs):
        pks = [phi_k(*job) for job in jobs]
        for pk, (a, b, c0, c1, first) in zip(pks, jobs):
            gp = _dot_tn(pk, x_v[a:b, :])
            if first:
                g_acc[c0:c1, :] = gp
            else:
                g_acc[c0:c1, :] += gp

    def phi_q(a, n):
        pq = _phi(_dot(x_v[pl.ds(a, n), :], wqp_v[...]))
        pq_v[pl.ds(a, n), :] = pq
        return pq

    def attention_stats(never):
        wait(grp1)
        start(grp3)
        key_stats((0, X1, 0, LANES, True), (0, X1, LANES, HALF, True))

        wait(grp2)
        start(grp4)
        key_stats((X1, X2, 0, LANES, False), (X1, X2, LANES, HALF, False))

        wait(grp3)
        start(grp5)
        key_stats((0, X2, HALF, D, True), (X2, X3, 0, HALF, False), (X2, X3, HALF, D, False))

        wait(grp4)
        wv_t = wv_v[...].T
        wq_t = wq_v[...].T
        pk = phi_k(X3, X4, 0, D, False)
        pk = jnp.concatenate([_after(never, wq_t, pk[0:D]), pk[D:]], axis=0)
        gp = _dot_tn(pk, x_v[X3:X4, :])
        g_acc[...] += gp
        g = g_acc[...] + _dot_tn(phi_k(X4, S, 0, D, False), x_v[X4:S, :])
        for c in range(NT):
            _scatter(g_s, c, g[:, _tile(c)])

        for c in range(NT):
            _scatter(wq_s, c, wq_t[:, _tile(c)].astype(F32))
            wqp_v[_tile(c), :] = _heads(wq_s, c, 0, H).reshape(D, LANES).astype(BF).T
        pq = jnp.concatenate([phi_q(a, QPRE) for a in range(0, S, TM)], axis=0)
        for c in range(NT):
            _scatter(wv_s, c, _after(never, pq[0:D, _tile(c)], wv_t[:, _tile(c)].astype(F32)))
            _scatter(wo_s, c, _after(never, gp[:, _tile(c)], wo_v[:, _tile(c)].astype(F32)))
        z = jnp.sum(z_acc[...], axis=0, keepdims=True)
        _scatter(z_s, 0, jnp.broadcast_to(z, (LANES, D)).T)
        zp_v[...] = _heads(z_s, 0, 0, H).reshape(D, LANES).T[0:SUBL, :]

        wait(grp5)

    def build_m(never):
        m = None
        for h0 in range(0, H, SUBL):
            for d in range(DH):
                r = d * PITCH + h0
                g = jnp.concatenate([g_s[c, r:r + SUBL, :] for c in range(NT)], axis=1)
                if m is not None:
                    g = _after(never, m, g)
                wv = jnp.concatenate([_heads(wv_s, c, h0, SUBL) for c in range(NT)], axis=2)
                kv = jnp.sum(g[None] * wv, axis=-1, keepdims=True)
                wo = jnp.concatenate([_heads(wo_s, c, h0, SUBL) for c in range(NT)], axis=2)
                m = jnp.sum(kv * wo, axis=0)
                m_v[d * H + h0:d * H + h0 + SUBL, :] = m.astype(BF)

    def normalized_q(r, n):
        pq = pq_v[pl.ds(r, n), :]
        t = pq * zp_v[0:1, :]
        t = (t[:, _tile(0)] + t[:, _tile(1)]) + (t[:, _tile(2)] + t[:, _tile(3)])
        t = t + pltpu.roll(t, 2 * H, 1)
        den = t + pltpu.roll(t, H, 1) + 1e-6
        inv = pl.reciprocal(den, approx=True)
        return (pq * jnp.concatenate([inv] * NT, axis=1)).astype(BF)

    def mix_rows(i, never):
        build_m(never)
        subs = []
        for s0 in range(0, TM, SUB):
            r = pl.multiple_of(i * TM + s0, SUB)
            xt = x_v[pl.ds(r, SUB), :]
            subs.append((s0, r, xt, _dot(xt, wg_v[...])))
        phi_q(pl.multiple_of(i * TM + QPRE, LANES), TM - QPRE)
        acts = []
        for s0, r, xt, pre in subs:
            gw = gw_v[...].astype(F32).reshape(1, D)
            logit = jnp.sum(xt.astype(F32) * gw, axis=-1, keepdims=True)
            gate = 1.0 / (1.0 + jnp.exp(-logit))
            up = _dot(xt, wu_v[...])
            sig = pl.reciprocal(1.0 + jnp.exp2(pre * -LOG2E), approx=True)
            acts.append((s0, r, gate, (pre * sig * up).astype(BF)))
        for s0, r, gate, act in acts:
            o = 0
            for n in (TAIL if s0 + SUB == TM else (SUB,)):
                rr = pl.multiple_of(r + o, 32)
                pqn = normalized_q(rr, n)
                g = gate[o:o + n]
                for c0, c1 in (LAST_COLS if s0 + o + n == TM else ((0, D),)):
                    a = _dot(pqn, m_v[:, c0:c1])
                    b = _dot(act[o:o + n, :], wd_v[:, c0:c1])
                    out_v[pl.ds(rr, n), c0:c1] = (g * a + (1.0 - g) * b).astype(BF)
                    ocopy(rr, n, c0, c1).start()
                o += n

    start(grp1)
    start(grp2)
    for slab in (wq_s, z_s, wv_s, wo_s):
        for d in range(DH):
            slab[:, d * PITCH + H:(d + 1) * PITCH, :] = jnp.zeros((slab.shape[0], PITCH - H, LANES), F32)

    def step(i, carry):
        @pl.when(i == 0)
        def _():
            attention_stats(never=i > 0)

        @pl.when(i > 0)
        def _():
            mix_rows(i - 1, never=i - 1 < 0)

        return carry

    lax.fori_loop(0, S // TM + 1, step, 0)
    ocopy(0, S, 0, D).wait()


@jax.jit
def pallas_gated_mix__linear_attn_block__swiglu_ffn__prompt_kernel(
    A_x: jax.Array,
    A_wqkv: jax.Array,
    A_wo: jax.Array,
    B_x: jax.Array,
    B_w_gate: jax.Array,
    B_w_up: jax.Array,
    B_w_down: jax.Array,
    gate_w: jax.Array,
):
    del B_x
    hbm = pl.BlockSpec(memory_space=pl.ANY)
    vmem = pltpu.VMEM
    slab = vmem((NT, DH * PITCH, LANES), F32)
    out = pl.pallas_call(
        _kernel,
        out_shape=jax.ShapeDtypeStruct((S, D), BF),
        in_specs=[hbm] * 7,
        out_specs=hbm,
        scratch_shapes=[
            vmem((S, D), BF),
            vmem((D, D), BF), vmem((D, D), BF), vmem((D, D), BF),
            vmem((D, D), BF),
            vmem((D, F), BF), vmem((D, F), BF), vmem((F, D), BF),
            vmem((D,), BF),
            vmem((S, D), BF),
            vmem((D, D), F32),
            vmem((SUBL, D), F32),
            vmem((D, D), BF),
            vmem((S, D), F32),
            vmem((SUBL, D), F32),
            vmem((D, D), BF),
            slab,
            vmem((1, DH * PITCH, LANES), F32),
            slab, slab, slab,
            pltpu.SemaphoreType.DMA((2,)),
        ],
        compiler_params=pltpu.CompilerParams(vmem_limit_bytes=64 * 1024 * 1024),
        name="gated_mix",
    )(A_x.reshape(S, D), A_wqkv, A_wo, B_w_gate, B_w_up, B_w_down, gate_w)
    return out.reshape(1, S, D)
```
